```python
import os as _os
_os.environ.setdefault("JAX_PLATFORMS", "cpu")
import jax
import jax.numpy as jnp

def _softmax(x, axis=-1):
    return jax.nn.softmax(x, axis=axis)
def _gelu(x):
    return jax.nn.gelu(x, approximate=True)
def _silu(x):
    return jax.nn.silu(x)
def _sigmoid(x):
    return jax.nn.sigmoid(x)
def _layernorm(x, axis=-1, eps=1e-5):
    m = jnp.mean(x, axis=axis, keepdims=True)
    v = jnp.var(x, axis=axis, keepdims=True)
    return (x - m) / jnp.sqrt(v + eps)
def _scatter_add(tgt, idx, src, axis=0):
    return tgt.at[idx].add(src)
def _segment_sum(src, seg, n):
    return jax.ops.segment_sum(src, seg, n)
class _Rng:
    def __init__(self, key):
        self._k = key
    def _next(self):
        self._k, sub = jax.random.split(self._k)
        return sub
    def normal(self, shape):
        return jax.random.normal(self._next(), shape, dtype=jnp.bfloat16)
    def randint(self, lo, hi, shape):
        return jax.random.randint(self._next(), shape, lo, hi, dtype=jnp.int32)
    def uniform(self, shape, lo=0.0, hi=1.0):
        return jax.random.uniform(self._next(), shape, jnp.bfloat16, lo, hi)
    def permutation(self, n):
        return jax.random.permutation(self._next(), n)


kernel_name = 'standalone__se_block__vision'

def setup_inputs():
    _rng = _Rng(jax.random.key(int.from_bytes(__import__("os").urandom(4), "little")))
    _w = (lambda a: (lambda t: t.astype(jnp.bfloat16) if jnp.issubdtype(t.dtype, jnp.floating) else t)(jnp.asarray(a)))
    H = W = 384
    C = 192; r = max(C // 16, 4)
    return {
        "x": _w((lambda *s: _rng.normal(s) * 0.8)(1, H, W, C)),
        "w_down": _w((lambda *s: _rng.normal(s) * 0.8)(C, r)),
        "w_up": _w((lambda *s: _rng.normal(s) * 0.8)(r, C)),
    }

def reference(x, w_down, w_up):
    s = x.mean(axis=(1, 2))
    s = _sigmoid(_silu(s @ w_down) @ w_up)
    return x * s[:, None, None, :]
```

```python
import jax
import jax.numpy as jnp
import jax.experimental.pallas as pl
import jax.experimental.pallas.tpu as pltpu


@jax.jit
def pallas_standalone__se_block__vision_kernel(
    x: jax.Array,
    w_down: jax.Array,
    w_up: jax.Array,
):
    _, H, W, C = x.shape
    R = w_down.shape[1]
    NS, UQ = 6, 4
    tail = (40, 15, 6, 2, 1)
    depth, rdepth = 4, 3
    CT, WT = C // 8, W // 128
    HS = H // NS
    NQ = HS * UQ
    CU = CT // UQ
    UR = CU * WT * 8
    inv_n = 1.0 / (H * W)

    chunks = [(a, 0, HS) for a in range(NS - 1)]
    r0 = 0
    for n in tail:
        chunks.append((NS - 1, r0, n))
        r0 += n
    assert r0 == HS
    NCH = len(chunks)

    def kernel(x_hbm, wd_hbm, wu_hbm, o_hbm, buf, wd_v, wu_v, wut_v, scale_v,
               rsem, wsem, osem):
        def rd(i):
            a, r0, n = chunks[i]
            sl = (a, pl.ds(r0 * UQ, n * UQ))
            return pltpu.make_async_copy(x_hbm.at[sl], buf.at[sl], rsem.at[i])

        rd(0).start()
        cwd = pltpu.make_async_copy(wd_hbm, wd_v, wsem.at[0])
        cwd.start()
        cwu = pltpu.make_async_copy(wu_hbm, wu_v, wsem.at[1])
        cwu.start()
        for i in range(1, rdepth):
            rd(i).start()
        cwd.wait()
        cwu.wait()
        wut_v[...] = wu_v[...].astype(jnp.float32).T.astype(jnp.bfloat16)

        acc = jnp.zeros((CT, 8, 128), jnp.float32)
        for i in range(NCH):
            a, r0, n = chunks[i]
            rd(i).wait()
            if i + rdepth < NCH:
                rd(i + rdepth).start()

            def body(h, acc, a=a):
                v = buf[a, pl.ds(h * UQ, UQ)].astype(jnp.float32).reshape(CT, WT, 8, 128)
                for t in range(WT):
                    acc = acc + v[:, t]
                return acc

            acc = jax.lax.fori_loop(r0, r0 + n, body, acc)

        tot = jnp.sum(acc.reshape(C, 128), axis=1, keepdims=True)
        mean = jnp.broadcast_to(tot * inv_n, (C, 128)).astype(jnp.bfloat16)
        h = jnp.dot(wd_v[...], mean, preferred_element_type=jnp.float32)
        h = h.astype(jnp.bfloat16).astype(jnp.float32)
        g = (h * jax.nn.sigmoid(h)).astype(jnp.bfloat16)
        z = jnp.dot(wut_v[...], g, preferred_element_type=jnp.float32)
        z = z.astype(jnp.bfloat16).astype(jnp.float32)
        s = jax.nn.sigmoid(z).astype(jnp.bfloat16).astype(jnp.float32)
        scale_v[...] = s.reshape(UQ, CU, 8, 128)

        def wr(q, slot):
            return pltpu.make_async_copy(buf.at[:, q], o_hbm.at[:, q], osem.at[slot])

        def body2(q, carry):
            sc = scale_v[q % UQ][:, None]
            for a in range(NS):
                v = buf[a, q].astype(jnp.float32).reshape(CU, WT, 8, 128)
                buf[a, q] = (v * sc).reshape(UR, 128).astype(jnp.bfloat16)
            slot = q % depth

            @pl.when(q >= depth)
            def _():
                wr(q - depth, slot).wait()

            wr(q, slot).start()
            return carry

        jax.lax.fori_loop(0, NQ, body2, 0)
        for q in range(NQ - depth, NQ):
            wr(q, q % depth).wait()

    xv = x.reshape(H, WT, 128, CT, 8).transpose(0, 3, 1, 4, 2).reshape(NS, NQ, UR, 128)
    out = pl.pallas_call(
        kernel,
        out_shape=jax.ShapeDtypeStruct(xv.shape, xv.dtype),
        in_specs=[pl.BlockSpec(memory_space=pl.ANY)] * 3,
        out_specs=pl.BlockSpec(memory_space=pl.ANY),
        scratch_shapes=[
            pltpu.VMEM(xv.shape, jnp.bfloat16),
            pltpu.VMEM((R, C), jnp.bfloat16),
            pltpu.VMEM((R, C), jnp.bfloat16),
            pltpu.VMEM((C, R), jnp.bfloat16),
            pltpu.VMEM((UQ, CU, 8, 128), jnp.float32),
            pltpu.SemaphoreType.DMA((NCH,)),
            pltpu.SemaphoreType.DMA((2,)),
            pltpu.SemaphoreType.DMA((depth,)),
        ],
        compiler_params=pltpu.CompilerParams(vmem_limit_bytes=64 * 1024 * 1024),
    )(xv, w_down.T, w_up)
    return out.reshape(H, CT, WT, 8, 128).transpose(0, 2, 4, 1, 3).reshape(1, H, W, C)
```

```python
import jax
import jax.numpy as jnp
import jax.experimental.pallas as pl
import jax.experimental.pallas.tpu as pltpu

F32, BF16 = jnp.float32, jnp.bfloat16

def _rnd(v):
    return v.astype(BF16).astype(F32)

def _sigmoid(v):
    d = _rnd(1.0 + _rnd(jnp.exp(-v)))
    return _rnd(pl.reciprocal(d, approx=True))

def _tree(terms):
    terms = list(terms)
    while len(terms) > 1:
        nxt = [terms[i] + terms[i + 1] for i in range(0, len(terms) - 1, 2)]
        if len(terms) % 2:
            nxt.append(terms[-1])
        terms = nxt
    return terms[0]

@jax.jit
def pallas_standalone__se_block__vision_kernel(x: jax.Array, w_down: jax.Array, w_up: jax.Array):
    cu, NU, NBR, UPR, lead, NB = 16, 22, 11, 2, 2, 4
    full, tail, fin, FG, nochk, nacc, prio = (9,), (8, 3, 1), (9, 2, 1), 4, True, 4, 0
    _, H, W, C = x.shape
    R = w_down.shape[1]
    CT, WT = C // 8, W // 128
    RR = CT * WT * 8
    MT = CT - FG
    MRW = MT * WT * 8
    FRW = FG * WT * 8
    TR = sum(tail)
    assert sum(fin) == TR
    UR = NU * cu
    B0 = UR
    L0 = UR + NBR
    assert L0 + sum(full) + TR == H
    K = len(full) + len(tail) + len(fin)
    assert NU - K >= K
    NUN = NBR * UPR
    BU = RR // UPR
    assert NUN <= NU and lead < NB
    inv_n = 1.0 / (H * W)
    NST, NQ, RUN = 54, 64, 64
    NA, NG, NP = 6, 9, 9
    assert NST * NQ * RUN == H * RR

    late = []
    r0 = L0
    for n in full:
        late.append((r0, n, 0, RR)); r0 += n
    T0 = r0
    for n in tail:
        late.append((r0, n, 0, MRW)); r0 += n
    r0 = T0
    for n in fin:
        late.append((r0, n, MRW, FRW)); r0 += n

    def kernel(x_hbm, wd_hbm, wu_hbm, o_hbm, buf, wd_v, wu_v, wdc_v, wub_v, tab_v, hp_v, sm,
               usem, lsem, wsem, osem, isem, bsem):
        def rdu(i, slot):
            sl = pl.ds(i * cu, cu)
            return pltpu.make_async_copy(x_hbm.at[sl], buf.at[sl], usem.at[slot])
        def rdl(j):
            r0, n, s0, sn = late[j]
            sl = (pl.ds(r0, n), pl.ds(s0, sn))
            return pltpu.make_async_copy(x_hbm.at[sl], buf.at[sl], lsem.at[j])
        xb = x_hbm.reshape(H * UPR, BU, 128)
        bb = buf.reshape(H * UPR, BU, 128)
        def bin_(k, slot):
            return pltpu.make_async_copy(xb.at[B0 * UPR + k], sm.at[slot], isem.at[slot])
        def bout(k, slot):
            return pltpu.make_async_copy(sm.at[slot], bb.at[B0 * UPR + k], bsem.at[slot])

        for i in range(K):
            rdu(i, i).start()
        for k in range(min(lead, NUN)):
            bin_(k, k).start(priority=prio)
        cwd = pltpu.make_async_copy(wd_hbm, wd_v, wsem.at[0]); cwd.start()
        cwu = pltpu.make_async_copy(wu_hbm, wu_v, wsem.at[1]); cwu.start()

        def service(i):
            if NUN == 0:
                return
            @pl.when(i < NUN)
            def _():
                s = jax.lax.rem(i, NB)
                bin_(i, s).wait()
                bout(i, s).start(priority=prio)
            k = i + lead
            @pl.when(k < NUN)
            def _():
                s = jax.lax.rem(k, NB)
                @pl.when(k >= NB)
                def _():
                    bout(k - NB, s).wait()
                bin_(k, s).start(priority=prio)

        def row(h, acc):
            v = buf[h].astype(F32).reshape(CT, WT, 8, 128)
            return acc + ((v[:, 0] + v[:, 1]) + v[:, 2])

        def loop_a(i, acc):
            slot = jax.lax.rem(i, K)
            rdu(i, slot).wait()
            rdu(i + K, slot).start()
            service(i)
            return jax.lax.fori_loop(i * cu, (i + 1) * cu, row, acc)
        acc = jax.lax.fori_loop(0, NU - K, loop_a, jnp.zeros((CT, 8, 128), F32))

        cwd.wait(); cwu.wait()
        wdt = wd_v[...].astype(F32)
        for c in range(FG * 8):
            wdc_v[c] = jnp.broadcast_to(wdt[:, MT * 8 + c:MT * 8 + c + 1], (R, 128))
        wut = wu_v[...].astype(F32).T
        for j in range(R):
            wub_v[j] = jnp.broadcast_to(wut[:, j:j + 1], (C, 128))

        def loop_b(i, acc):
            rdu(i, jax.lax.rem(i, K)).wait()
            for j in range(K):
                @pl.when(i == NU - K + j)
                def _():
                    rdl(j).start()
            service(i)
            return jax.lax.fori_loop(i * cu, (i + 1) * cu, row, acc)
        acc = jax.lax.fori_loop(NU - K, NU, loop_b, acc)

        for k in range(max(0, NUN - NB), NUN):
            bout(k, k % NB).wait()
        acc = jax.lax.fori_loop(B0, L0, row, acc)
        for j in range(len(full)):
            r0, n, _, _ = late[j]
            rdl(j).wait()
            acc = jax.lax.fori_loop(r0, r0 + n, row, acc)

        accm, accf = acc[:MT], acc[MT:]
        def rowm(h, a):
            v = buf[h, pl.ds(0, MRW)].astype(F32).reshape(MT, WT, 8, 128)
            return a + ((v[:, 0] + v[:, 1]) + v[:, 2])
        for j in range(len(full), len(full) + len(tail)):
            r0, n, _, _ = late[j]
            rdl(j).wait()
            accm = jax.lax.fori_loop(r0, r0 + n, rowm, accm)
        totm = jnp.sum(accm.reshape(MT * 8, 128), axis=1, keepdims=True)
        meanm = jnp.broadcast_to(totm * inv_n, (MT * 8, 128)).astype(BF16)
        hp_v[...] = jnp.dot(wd_v[:, pl.ds(0, MT * 8)], meanm, preferred_element_type=F32)

        for j in range(len(full) + len(tail), K):
            r0, n, _, _ = late[j]
            rdl(j).wait()
            parts = [accf] + [None] * (nacc - 1)
            k = 1
            for r in range(n):
                v = buf[r0 + r, pl.ds(MRW, FRW)].astype(F32).reshape(FG, WT, 8, 128)
                for t in range(WT):
                    p = k % nacc
                    parts[p] = v[:, t] if parts[p] is None else parts[p] + v[:, t]
                    k += 1
            accf = _tree([p for p in parts if p is not None])
        totf = jnp.sum(accf.reshape(FG * 8, 128), axis=1, keepdims=True)
        meanf = _rnd(jnp.broadcast_to(totf * inv_n, (FG * 8, 128)))
        h = _rnd(_tree([wdc_v[c] * meanf[c:c + 1, :] for c in range(FG * 8)]) + hp_v[...])
        g = _rnd(h * _sigmoid(h))
        gb = [jnp.broadcast_to(g[j:j + 1, :], (8, 128)) for j in range(R)]

        buf1 = buf.reshape(NST, NQ, RUN, 128)
        buf9 = buf.reshape(NA, NP, NQ, RUN, 128)
        o9 = o_hbm.reshape(NA, NP, NQ, RUN, 128)

        stile = {}
        def get_s(ct):
            if ct not in stile:
                z = _rnd(_tree([wub_v[j, pl.ds(ct * 8, 8), :] * gb[j] for j in range(R)]))
                stile[ct] = _sigmoid(z)
            return stile[ct]
        for p in range(NP):
            sc = jnp.stack([get_s((8 * p + i) // WT) for i in range(8)])
            for a in range(NA):
                v = buf9[a, p, 0].astype(F32).reshape(8, 8, 128)
                buf9[a, p, 0] = (v * sc).reshape(RUN, 128).astype(BF16)
            pltpu.make_async_copy(buf9.at[:, p, 0], o9.at[:, p, 0], osem.at[p]).start()
            tab_v[p] = sc

        def wr(g, q, slot):
            sl = (pl.ds(g * NA, NA), q)
            return pltpu.make_async_copy(buf1.at[sl], o_hbm.at[sl], osem.at[slot])

        def body_g(g, carry):
            def body_q(q, carry):
                for a in range(NA):
                    st = g * NA + a
                    m = jax.lax.rem(st + q, NP)
                    v = buf1[st, q].astype(F32).reshape(8, 8, 128)
                    buf1[st, q] = (v * tab_v[m]).reshape(RUN, 128).astype(BF16)
                slot = jax.lax.rem(q - 1, NP)
                wr(g, q, slot).wait()
                wr(g, q, slot).start()
                return carry
            return jax.lax.fori_loop(1, NQ, body_q, carry)
        jax.lax.fori_loop(0, NG, body_g, 0)
        for p in range(NP):
            wr(NG - 1, NQ - NP + p, p).wait()

    xv = x.reshape(H, WT, 128, CT, 8).transpose(0, 3, 1, 4, 2).reshape(H, RR, 128)
    out = pl.pallas_call(
        kernel,
        out_shape=jax.ShapeDtypeStruct((NST, NQ, RUN, 128), xv.dtype),
        in_specs=[pl.BlockSpec(memory_space=pl.ANY)] * 3,
        out_specs=pl.BlockSpec(memory_space=pl.ANY),
        scratch_shapes=[
            pltpu.VMEM(xv.shape, BF16),
            pltpu.VMEM((R, C), BF16),
            pltpu.VMEM((R, C), BF16),
            pltpu.VMEM((FG * 8, R, 128), F32),
            pltpu.VMEM((R, C, 128), F32),
            pltpu.VMEM((NP, 8, 8, 128), F32),
            pltpu.VMEM((R, 128), F32),
            pltpu.SMEM((NB, BU, 128), BF16),
            pltpu.SemaphoreType.DMA((K,)),
            pltpu.SemaphoreType.DMA((K,)),
            pltpu.SemaphoreType.DMA((2,)),
            pltpu.SemaphoreType.DMA((NP,)),
            pltpu.SemaphoreType.DMA((NB,)),
            pltpu.SemaphoreType.DMA((NB,)),
        ],
        compiler_params=pltpu.CompilerParams(vmem_limit_bytes=64 * 1024 * 1024,
            disable_bounds_checks=nochk, disable_semaphore_checks=nochk),
    )(xv, w_down.T, w_up)
    return out.reshape(H, CT, WT, 8, 128).transpose(0, 2, 4, 1, 3).reshape(1, H, W, C)
```

```python
import jax
import jax.numpy as jnp
import jax.experimental.pallas as pl
import jax.experimental.pallas.tpu as pltpu

F32, BF16 = jnp.float32, jnp.bfloat16
_NEG_LOG2E = -1.4426950408889634


def _rnd(v):
    return v.astype(BF16).astype(F32)


def _sigmoid(v):
    d = _rnd(1.0 + _rnd(jnp.exp2(v * _NEG_LOG2E)))
    return _rnd(pl.reciprocal(d, approx=True))


def _tree(terms):
    terms = list(terms)
    while len(terms) > 1:
        nxt = [terms[i] + terms[i + 1] for i in range(0, len(terms) - 1, 2)]
        if len(terms) % 2:
            nxt.append(terms[-1])
        terms = nxt
    return terms[0]


@jax.jit
def pallas_standalone__se_block__vision_kernel(
    x: jax.Array,
    w_down: jax.Array,
    w_up: jax.Array,
):
    B, H, W, C = x.shape
    R = w_down.shape[1]
    CT, WT = C // 8, W // 128
    inv_n = 1.0 / (H * W)

    RUN = 64
    NQ = 64
    NP = CT * WT // 8
    NST = H * NP // NQ
    assert B == 1 and C % 8 == 0 and W % 128 == 0
    assert NP * 8 == CT * WT and NST * NQ == H * NP and NQ % NP == 1

    T, F = 2 * NP, 2
    G = NST // T
    PPQ = 4
    KR = RUN // PPQ
    MQ = NQ - 1
    NI = G * MQ
    DQ, LQ, CL = 6, 1, 2
    FQ = LQ + CL + 1
    TABQ = 40
    ST1 = 4
    T1 = 8 * (ST1 + 1) // WT
    T2 = 8 * (NP - 1) // WT
    NA = NST // NP
    FIRST = 2
    assert G * T == NST and NA * NP == NST and DQ * PPQ > NP

    def kernel(x_hbm, wd_hbm, wu_hbm, o_hbm,
               buf, wd_v, wu_v, wd2_v, wdc_v, wub_v, hp_v, m2_v, tab_v,
               bsem, fsem, lsem, wsem, osem):
        buf1 = buf.reshape(NST, NQ, RUN, 128)
        buf9 = buf.reshape(NA, NP, NQ, RUN, 128)
        x9 = x_hbm.reshape(NA, NP, NQ, RUN, 128)
        o9 = o_hbm.reshape(NA, NP, NQ, RUN, 128)

        def split(i):
            if isinstance(i, int):
                return i // MQ, i % MQ
            return jax.lax.div(i, MQ), jax.lax.rem(i, MQ)

        def lo(gq, r, slot):
            s = (gq[0], pl.ds(0, T - F), gq[1], r)
            return pltpu.make_async_copy(x_hbm.at[s], buf.at[s], bsem.at[slot * PPQ + r])

        def hi(gq, r, slot):
            s = (gq[0], pl.ds(T - F, F), gq[1], r)
            return pltpu.make_async_copy(x_hbm.at[s], buf.at[s], fsem.at[slot * PPQ + r])

        def fin(p, a0, a1, k):
            s = (pl.ds(a0, a1 - a0), p, MQ)
            return pltpu.make_async_copy(x9.at[s], buf9.at[s], lsem.at[k])

        for j in range(LQ):
            for r in range(PPQ):
                lo((0, j), r, j).start(priority=1)
                hi((0, j), r, j).start(priority=0)

        def fill(j, carry):
            for r in range(PPQ):
                lo((0, j), r, j).start(priority=1)
            return carry

        jax.lax.fori_loop(LQ, DQ, fill, 0)
        cwd = pltpu.make_async_copy(wd_hbm, wd_v, wsem.at[0])
        cwu = pltpu.make_async_copy(wu_hbm, wu_v, wsem.at[1])
        cwd.start()
        cwu.start()

        def step(i, acc, *, dma, drain, comp):
            acc = list(acc)
            if dma:
                cur, lo_next, hi_next = split(i), split(i + DQ), split(i + LQ)
                lo_slot = jax.lax.rem(i, DQ)
                hi_slot = jax.lax.rem(i + LQ, FQ)
            if comp:
                old = split(i - CL)
                old_slot = jax.lax.rem(i - CL, FQ)
                q9 = jax.lax.rem(old[1], NP)
                stripe = [jnp.where(m < q9, m + NP - q9, m - q9) for m in range(NP)]
            for r in range(PPQ):
                if dma:
                    lo(cur, r, lo_slot).wait()
                if dma and not drain:
                    lo(lo_next, r, lo_slot).start(priority=1)
                    hi(hi_next, r, hi_slot).start(priority=0)
                if dma and drain:
                    k = (i + DQ - NI) * PPQ + r

                    @pl.when(k < NP - 1)
                    def _():
                        fin(k, 0, NA, k).start(priority=1)

                    if r == (NP - 1) % PPQ:
                        @pl.when(k == NP - 1)
                        def _():
                            fin(NP - 1, 0, NA - 1, NP - 1).start(priority=1)

                    if r == NP % PPQ:
                        @pl.when(k == NP)
                        def _():
                            fin(NP - 1, NA - 1, NA, NP).start(priority=1)

                    @pl.when(i + LQ < NI)
                    def _():
                        hi(hi_next, r, hi_slot).start(priority=0)

                if comp:
                    hi(old, r, old_slot).wait()
                    for m in range(NP):
                        v = _tree([
                            buf[old[0], stripe[m] + d * NP, old[1], r]
                            .astype(F32).reshape(KR // 8, 8, 128)
                            for d in range(T // NP)])
                        for t in range(KR // 8):
                            ct = (8 * m + (KR // 8) * r + t) // WT
                            acc[ct] = acc[ct] + v[t]
            return tuple(acc)

        def steps(lo_i, hi_i, acc, **mode):
            return jax.lax.fori_loop(lo_i, hi_i, lambda i, a: step(i, a, **mode), acc)

        steps(0, CL, (), dma=True, drain=False, comp=False)
        acc = tuple(jnp.zeros((8, 128), F32) for _ in range(CT))
        acc = steps(CL, TABQ, acc, dma=True, drain=False, comp=True)

        cwd.wait()
        cwu.wait()
        wdt = wd_v[...].astype(F32)
        wd2_v[...] = wdt[:, T1 * 8:T2 * 8].astype(BF16)
        for c in range((CT - T2) * 8):
            wdc_v[c] = jnp.broadcast_to(wdt[:, T2 * 8 + c:T2 * 8 + c + 1], (R, 128))
        wut = wu_v[...].astype(F32).T
        for j in range(R):
            wub_v[j] = jnp.broadcast_to(wut[:, j:j + 1], (C, 128))

        acc = steps(TABQ, NI - DQ, acc, dma=True, drain=False, comp=True)
        acc = steps(NI - DQ, NI, acc, dma=True, drain=True, comp=True)
        acc = steps(NI, NI + CL, acc, dma=False, drain=False, comp=True)
        acc = list(acc)

        def add_fin(p, a0, a1, k):
            fin(p, a0, a1, k).wait()
            v = _tree([buf9[a, p, MQ].astype(F32).reshape(8, 8, 128)
                       for a in range(a0, a1)])
            for ct in sorted({(8 * p + i) // WT for i in range(8)}):
                acc[ct] = _tree([acc[ct]] + [v[i] for i in range(8)
                                             if (8 * p + i) // WT == ct])

        def means(t0, t1):
            a = jnp.stack(acc[t0:t1]).reshape((t1 - t0) * 8, 128)
            tot = jnp.sum(a, axis=1, keepdims=True)
            return jnp.broadcast_to(tot * inv_n, a.shape)

        for p in range(NP - 1):
            add_fin(p, 0, NA, p)
            if p == ST1:
                hp_v[...] = jnp.dot(wd_v[:, pl.ds(0, T1 * 8)], means(0, T1).astype(BF16),
                                    preferred_element_type=F32)
        m2_v[...] = means(T1, T2).astype(BF16)
        add_fin(NP - 1, 0, NA - 1, NP - 1)
        add_fin(NP - 1, NA - 1, NA, NP)

        hp = hp_v[...] + jnp.dot(wd2_v[...], m2_v[...], preferred_element_type=F32)
        m3 = _rnd(means(T2, CT))
        h = _rnd(_tree([wdc_v[c] * m3[c:c + 1, :] for c in range((CT - T2) * 8)]) + hp)
        g = _rnd(h * _sigmoid(h))
        gb = [jnp.broadcast_to(g[j:j + 1, :], (8, 128)) for j in range(R)]

        scale = {}

        def scale_tile(ct):
            if ct not in scale:
                z = _tree([wub_v[j, pl.ds(ct * 8, 8), :] * gb[j] for j in range(R)])
                scale[ct] = _sigmoid(_rnd(z))
            return scale[ct]

        for p in range(NP):
            sc = jnp.stack([scale_tile((8 * p + i) // WT) for i in range(8)])
            cuts = (0, FIRST, NA) if p == 0 else (0, NA)
            for a0, a1 in zip(cuts, cuts[1:]):
                for a in range(a0, a1):
                    v = buf9[a, p, 0].astype(F32).reshape(8, 8, 128)
                    buf9[a, p, 0] = (v * sc).reshape(RUN, 128).astype(BF16)
                s = (pl.ds(a0, a1 - a0), p, 0)
                pltpu.make_async_copy(buf9.at[s], o9.at[s], osem.at[p]).start()
            tab_v[p] = sc

        def wr(gi, q, slot):
            s = (pl.ds(gi * NA, NA), q)
            return pltpu.make_async_copy(buf1.at[s], o_hbm.at[s], osem.at[slot])

        def out_group(gi, carry):
            def out_run(q, carry):
                for a in range(NA):
                    st = gi * NA + a
                    v = buf1[st, q].astype(F32).reshape(8, 8, 128)
                    sc = tab_v[jax.lax.rem(st + q, NP)]
                    buf1[st, q] = (v * sc).reshape(RUN, 128).astype(BF16)
                slot = jax.lax.rem(q - 1, NP)
                wr(gi, q, slot).wait()
                wr(gi, q, slot).start()
                return carry

            return jax.lax.fori_loop(1, NQ, out_run, carry)

        jax.lax.fori_loop(0, NP, out_group, 0)
        for p in range(NP):
            wr(NP - 1, NQ - NP + p, p).wait()

    xv = x.reshape(H, WT, 128, CT, 8).transpose(0, 3, 1, 4, 2).reshape(G, T, NQ, PPQ, KR, 128)
    out = pl.pallas_call(
        kernel,
        out_shape=jax.ShapeDtypeStruct((NST, NQ, RUN, 128), x.dtype),
        in_specs=[pl.BlockSpec(memory_space=pl.ANY)] * 3,
        out_specs=pl.BlockSpec(memory_space=pl.ANY),
        scratch_shapes=[
            pltpu.VMEM(xv.shape, BF16),
            pltpu.VMEM((R, C), BF16),
            pltpu.VMEM((R, C), BF16),
            pltpu.VMEM((R, (T2 - T1) * 8), BF16),
            pltpu.VMEM(((CT - T2) * 8, R, 128), F32),
            pltpu.VMEM((R, C, 128), F32),
            pltpu.VMEM((R, 128), F32),
            pltpu.VMEM(((T2 - T1) * 8, 128), BF16),
            pltpu.VMEM((NP, 8, 8, 128), F32),
            pltpu.SemaphoreType.DMA((DQ * PPQ,)),
            pltpu.SemaphoreType.DMA((FQ * PPQ,)),
            pltpu.SemaphoreType.DMA((NP + 1,)),
            pltpu.SemaphoreType.DMA((2,)),
            pltpu.SemaphoreType.DMA((NP,)),
        ],
        compiler_params=pltpu.CompilerParams(
            vmem_limit_bytes=64 * 1024 * 1024,
            disable_bounds_checks=True,
            disable_semaphore_checks=True,
        ),
    )(xv, w_down.T, w_up)
    return out.reshape(H, CT, WT, 8, 128).transpose(0, 2, 4, 1, 3).reshape(B, H, W, C)
```

```python
import jax
import jax.numpy as jnp
import jax.experimental.pallas as pl
import jax.experimental.pallas.tpu as pltpu

F32, BF16 = jnp.float32, jnp.bfloat16
_NEG_LOG2E = -1.4426950408889634


def _rnd(v):
    return v.astype(BF16).astype(F32)


def _sigmoid(v):
    d = _rnd(1.0 + _rnd(jnp.exp2(v * _NEG_LOG2E)))
    return _rnd(pl.reciprocal(d, approx=True))


def _tree(terms):
    terms = list(terms)
    while len(terms) > 1:
        nxt = [terms[i] + terms[i + 1] for i in range(0, len(terms) - 1, 2)]
        if len(terms) % 2:
            nxt.append(terms[-1])
        terms = nxt
    return terms[0]


@jax.jit
def pallas_standalone__se_block__vision_kernel(
    x: jax.Array,
    w_down: jax.Array,
    w_up: jax.Array,
):
    B, H, W, C = x.shape
    R = w_down.shape[1]
    CT, WT = C // 8, W // 128
    inv_n = 1.0 / (H * W)

    RUN = 64
    NQ = 64
    NP = CT * WT // 8
    NST = H * NP // NQ
    assert B == 1 and C % 8 == 0 and W % 128 == 0
    assert NP * 8 == CT * WT and NST * NQ == H * NP and NQ % NP == 1

    T, F = 2 * NP, 2
    G = NST // T
    PPQ = 4
    KR = RUN // PPQ
    MQ = NQ - 1
    NI = G * MQ
    DQ, LQ, CL = 6, 1, 2
    FQ = LQ + CL + 1
    TABQ = 40
    ST1 = 4
    T1 = 8 * (ST1 + 1) // WT
    T2 = 8 * (NP - 1) // WT
    NA = 2 * G
    assert G * T == NST and T % NA == 0 and DQ * PPQ > NP

    def kernel(x_hbm, wd_hbm, wu_hbm, o_hbm,
               buf, wd_v, wu_v, wd2_v, wdc_v, wub_v, hp_v, m2_v, tab_v,
               bsem, fsem, lsem, wsem, osem):
        def split(i):
            if isinstance(i, int):
                return i // MQ, i % MQ
            return jax.lax.div(i, MQ), jax.lax.rem(i, MQ)

        def lo(gq, r, slot):
            s = (gq[0], pl.ds(0, T - F), gq[1], pl.ds(r * KR, KR))
            return pltpu.make_async_copy(x_hbm.at[s], buf.at[s], bsem.at[slot * PPQ + r])

        def hi(gq, r, slot):
            s = (gq[0], pl.ds(T - F, F), gq[1], pl.ds(r * KR, KR))
            return pltpu.make_async_copy(x_hbm.at[s], buf.at[s], fsem.at[slot * PPQ + r])

        def fin(st, g0, g1, k):
            s = (pl.ds(g0, g1 - g0), st, MQ)
            return pltpu.make_async_copy(x_hbm.at[s], buf.at[s], lsem.at[k])

        for j in range(LQ):
            for r in range(PPQ):
                lo((0, j), r, j).start(priority=1)
                hi((0, j), r, j).start(priority=0)

        def fill(j, carry):
            for r in range(PPQ):
                lo((0, j), r, j).start(priority=1)
            return carry

        jax.lax.fori_loop(LQ, DQ, fill, 0)
        cwd = pltpu.make_async_copy(wd_hbm, wd_v, wsem.at[0])
        cwu = pltpu.make_async_copy(wu_hbm, wu_v, wsem.at[1])
        cwd.start()
        cwu.start()

        def step(i, acc, *, dma, drain, comp):
            acc = list(acc)
            if dma:
                cur, lo_next, hi_next = split(i), split(i + DQ), split(i + LQ)
                lo_slot = jax.lax.rem(i, DQ)
                hi_slot = jax.lax.rem(i + LQ, FQ)
            if comp:
                old = split(i - CL)
                old_slot = jax.lax.rem(i - CL, FQ)
                q9 = jax.lax.rem(old[1], NP)
                stripe = [jnp.where(m < q9, m + NP - q9, m - q9) for m in range(NP)]
            for r in range(PPQ):
                if dma:
                    lo(cur, r, lo_slot).wait()
                if dma and not drain:
                    lo(lo_next, r, lo_slot).start(priority=1)
                    hi(hi_next, r, hi_slot).start(priority=0)
                if dma and drain:
                    k = (i + DQ - NI) * PPQ + r

                    @pl.when(k < NP - 1)
                    def _():
                        fin(k, 0, G, k).start(priority=1)
                        fin(k + NP, 0, G, k + NP).start(priority=1)

                    if r == (NP - 1) % PPQ:
                        @pl.when(k == NP - 1)
                        def _():
                            fin(NP - 1, 0, G, NP - 1).start(priority=1)
                            fin(T - 1, 0, G - 1, T - 1).start(priority=1)

                    if r == NP % PPQ:
                        @pl.when(k == NP)
                        def _():
                            fin(T - 1, G - 1, G, T).start(priority=1)

                    @pl.when(i + LQ < NI)
                    def _():
                        hi(hi_next, r, hi_slot).start(priority=0)

                if comp:
                    hi(old, r, old_slot).wait()
                    for m in range(NP):
                        v = _tree([
                            buf[old[0], stripe[m] + d * NP, old[1], pl.ds(r * KR, KR)]
                            .astype(F32).reshape(KR // 8, 8, 128)
                            for d in range(T // NP)])
                        for t in range(KR // 8):
                            ct = (8 * m + (KR // 8) * r + t) // WT
                            acc[ct] = acc[ct] + v[t]
            return tuple(acc)

        def steps(lo_i, hi_i, acc, **mode):
            return jax.lax.fori_loop(lo_i, hi_i, lambda i, a: step(i, a, **mode), acc)

        steps(0, CL, (), dma=True, drain=False, comp=False)
        acc = tuple(jnp.zeros((8, 128), F32) for _ in range(CT))
        acc = steps(CL, TABQ, acc, dma=True, drain=False, comp=True)

        cwd.wait()
        cwu.wait()
        wdt = wd_v[...].astype(F32)
        wd2_v[...] = wdt[:, T1 * 8:T2 * 8].astype(BF16)
        for c in range((CT - T2) * 8):
            wdc_v[c] = jnp.broadcast_to(wdt[:, T2 * 8 + c:T2 * 8 + c + 1], (R, 128))
        wut = wu_v[...].astype(F32).T
        for j in range(R):
            wub_v[j] = jnp.broadcast_to(wut[:, j:j + 1], (C, 128))

        acc = steps(TABQ, NI - DQ, acc, dma=True, drain=False, comp=True)
        acc = steps(NI - DQ, NI, acc, dma=True, drain=True, comp=True)
        acc = steps(NI, NI + CL, acc, dma=False, drain=False, comp=True)
        acc = list(acc)

        def add_fin(p, *copies):
            for c in copies:
                fin(*c).wait()
            v = _tree([buf[gi, st, MQ].astype(F32).reshape(8, 8, 128)
                       for st, g0, g1, _ in copies for gi in range(g0, g1)])
            for ct in sorted({(8 * p + i) // WT for i in range(8)}):
                acc[ct] = _tree([acc[ct]] + [v[i] for i in range(8)
                                             if (8 * p + i) // WT == ct])

        def means(t0, t1):
            a = jnp.stack(acc[t0:t1]).reshape((t1 - t0) * 8, 128)
            tot = jnp.sum(a, axis=1, keepdims=True)
            return jnp.broadcast_to(tot * inv_n, a.shape)

        for p in range(NP - 1):
            add_fin(p, (p, 0, G, p), (p + NP, 0, G, p + NP))
            if p == ST1:
                hp_v[...] = jnp.dot(wd_v[:, pl.ds(0, T1 * 8)], means(0, T1).astype(BF16),
                                    preferred_element_type=F32)
        m2_v[...] = means(T1, T2).astype(BF16)
        add_fin(NP - 1, (NP - 1, 0, G, NP - 1), (T - 1, 0, G - 1, T - 1))
        add_fin(NP - 1, (T - 1, G - 1, G, T))

        hp = hp_v[...] + jnp.dot(wd2_v[...], m2_v[...], preferred_element_type=F32)
        m3 = _rnd(means(T2, CT))
        h = _rnd(_tree([wdc_v[c] * m3[c:c + 1, :] for c in range((CT - T2) * 8)]) + hp)
        g = _rnd(h * _sigmoid(h))
        gb = [jnp.broadcast_to(g[j:j + 1, :], (8, 128)) for j in range(R)]

        scale = {}

        def scale_tile(ct):
            if ct not in scale:
                z = _tree([wub_v[j, pl.ds(ct * 8, 8), :] * gb[j] for j in range(R)])
                scale[ct] = _sigmoid(_rnd(z))
            return scale[ct]

        for p in range(NP):
            sc = jnp.stack([scale_tile((8 * p + i) // WT) for i in range(8)])
            for st in (p, p + NP):
                for gi in range(G):
                    v = buf[gi, st, 0].astype(F32).reshape(8, 8, 128)
                    buf[gi, st, 0] = (v * sc).reshape(RUN, 128).astype(BF16)
                pltpu.make_async_copy(buf.at[:, st, 0], o_hbm.at[:, st, 0], osem.at[p]).start()
            tab_v[p] = sc

        def wr(gi, st0, q, slot):
            s = (gi, pl.ds(st0, NA), q)
            return pltpu.make_async_copy(buf.at[s], o_hbm.at[s], osem.at[slot])

        def out_stripes(n, carry):
            gi = jax.lax.div(n, T // NA)
            st0 = jax.lax.rem(n, T // NA) * NA

            def out_run(q, carry):
                for a in range(NA):
                    v = buf[gi, st0 + a, q].astype(F32).reshape(8, 8, 128)
                    sc = tab_v[jax.lax.rem(st0 + a + q, NP)]
                    buf[gi, st0 + a, q] = (v * sc).reshape(RUN, 128).astype(BF16)
                slot = jax.lax.rem(q - 1, NP)
                wr(gi, st0, q, slot).wait()
                wr(gi, st0, q, slot).start()
                return carry

            return jax.lax.fori_loop(1, NQ, out_run, carry)

        jax.lax.fori_loop(0, NST // NA, out_stripes, 0)
        for p in range(NP):
            wr(G - 1, T - NA, NQ - NP + p, p).wait()

    xv = x.reshape(H, WT, 128, CT, 8).transpose(0, 3, 1, 4, 2).reshape(G, T, NQ, RUN, 128)
    out = pl.pallas_call(
        kernel,
        out_shape=jax.ShapeDtypeStruct(xv.shape, xv.dtype),
        in_specs=[pl.BlockSpec(memory_space=pl.ANY)] * 3,
        out_specs=pl.BlockSpec(memory_space=pl.ANY),
        scratch_shapes=[
            pltpu.VMEM(xv.shape, BF16),
            pltpu.VMEM((R, C), BF16),
            pltpu.VMEM((R, C), BF16),
            pltpu.VMEM((R, (T2 - T1) * 8), BF16),
            pltpu.VMEM(((CT - T2) * 8, R, 128), F32),
            pltpu.VMEM((R, C, 128), F32),
            pltpu.VMEM((R, 128), F32),
            pltpu.VMEM(((T2 - T1) * 8, 128), BF16),
            pltpu.VMEM((NP, 8, 8, 128), F32),
            pltpu.SemaphoreType.DMA((DQ * PPQ,)),
            pltpu.SemaphoreType.DMA((FQ * PPQ,)),
            pltpu.SemaphoreType.DMA((T + 1,)),
            pltpu.SemaphoreType.DMA((2,)),
            pltpu.SemaphoreType.DMA((NP,)),
        ],
        compiler_params=pltpu.CompilerParams(
            vmem_limit_bytes=64 * 1024 * 1024,
            disable_bounds_checks=True,
            disable_semaphore_checks=True,
        ),
    )(xv, w_down.T, w_up)
    return out.reshape(H, CT, WT, 8, 128).transpose(0, 2, 4, 1, 3).reshape(B, H, W, C)
```

```python
import jax
import jax.numpy as jnp
import jax.experimental.pallas as pl
import jax.experimental.pallas.tpu as pltpu

F32, BF16 = jnp.float32, jnp.bfloat16
_NEG_LOG2E = -1.4426950408889634


def _rnd(v):
    return v.astype(BF16).astype(F32)


def _sigmoid(v):
    d = _rnd(1.0 + _rnd(jnp.exp2(v * _NEG_LOG2E)))
    return _rnd(pl.reciprocal(d, approx=True))


def _tree(terms):
    terms = list(terms)
    while len(terms) > 1:
        nxt = [terms[i] + terms[i + 1] for i in range(0, len(terms) - 1, 2)]
        if len(terms) % 2:
            nxt.append(terms[-1])
        terms = nxt
    return terms[0]


@jax.jit
def pallas_standalone__se_block__vision_kernel(
    x: jax.Array,
    w_down: jax.Array,
    w_up: jax.Array,
):
    B, H, W, C = x.shape
    R = w_down.shape[1]
    CT, WT = C // 8, W // 128
    inv_n = 1.0 / (H * W)

    RUN = 64
    NQ = 64
    NP = CT * WT // 8
    NST = H * NP // NQ
    assert B == 1 and C % 8 == 0 and W % 128 == 0
    assert NP * 8 == CT * WT and NST * NQ == H * NP and NQ % NP == 1

    T, F = 2 * NP, 2
    G = NST // T
    PPQ = 4
    KR = RUN // PPQ
    MQ = NQ - 1
    NI = G * MQ
    DQ, LQ, CL = 6, 1, 2
    FQ = LQ + CL + 1
    TABQ = 40
    ST1 = 4
    T1 = 8 * (ST1 + 1) // WT
    T2 = 8 * (NP - 1) // WT
    NA = 2 * G
    assert G * T == NST and T % NA == 0
    assert LQ == 1 and DQ > PPQ and DQ * PPQ > NP

    def kernel(x_hbm, wd_hbm, wu_hbm, o_hbm,
               buf, wd_v, wu_v, wd2_v, wdc_v, wub_v, hp_v, m2_v, tab_v,
               bsem, fsem, lsem, wsem, osem):
        def split(i):
            return jax.lax.div(i, MQ), jax.lax.rem(i, MQ)

        def lo(gq, r, slot):
            s = (gq[0], pl.ds(0, T - F), gq[1], pl.ds(r * KR, KR))
            return pltpu.make_async_copy(x_hbm.at[s], buf.at[s], bsem.at[slot * PPQ + r])

        def hi(gq, r, slot):
            s = (gq[0], pl.ds(T - F, F), gq[1], pl.ds(r * KR, KR))
            return pltpu.make_async_copy(x_hbm.at[s], buf.at[s], fsem.at[slot * PPQ + r])

        def fin(st, g0, g1, k):
            s = (pl.ds(g0, g1 - g0), st, MQ)
            return pltpu.make_async_copy(x_hbm.at[s], buf.at[s], lsem.at[k])

        for r in range(PPQ):
            lo((0, 0), r, 0).start(priority=1)

        def fill(j, carry):
            for r in range(PPQ):
                lo((0, j), r, j).start(priority=1)
            for r in range(PPQ):
                @pl.when(j == r + 1)
                def _():
                    hi((0, 0), r, 0).start(priority=0)
            return carry

        jax.lax.fori_loop(1, DQ, fill, 0)
        cwd = pltpu.make_async_copy(wd_hbm, wd_v, wsem.at[0])
        cwu = pltpu.make_async_copy(wu_hbm, wu_v, wsem.at[1])
        cwd.start()
        cwu.start()

        def step(i, acc, *, dma, drain, comp):
            acc = list(acc)
            if dma:
                cur, lo_next, hi_next = split(i), split(i + DQ), split(i + LQ)
                lo_slot = jax.lax.rem(i, DQ)
                hi_slot = jax.lax.rem(i + LQ, FQ)
            if comp:
                old = split(i - CL)
                old_slot = jax.lax.rem(i - CL, FQ)
                q9 = jax.lax.rem(old[1], NP)
                stripe = [jnp.where(m < q9, m + NP - q9, m - q9) for m in range(NP)]
            for r in range(PPQ):
                if dma:
                    lo(cur, r, lo_slot).wait()
                if dma and not drain:
                    lo(lo_next, r, lo_slot).start(priority=1)
                    hi(hi_next, r, hi_slot).start(priority=0)
                if dma and drain:
                    k = (i + DQ - NI) * PPQ + r

                    @pl.when(k < NP - 1)
                    def _():
                        fin(k, 0, G, k).start(priority=1)
                        fin(k + NP, 0, G, k + NP).start(priority=1)

                    if r == (NP - 1) % PPQ:
                        @pl.when(k == NP - 1)
                        def _():
                            fin(NP - 1, 0, G, NP - 1).start(priority=1)
                            fin(T - 1, 0, G - 1, T - 1).start(priority=1)

                    if r == NP % PPQ:
                        @pl.when(k == NP)
                        def _():
                            fin(T - 1, G - 1, G, T).start(priority=1)

                    @pl.when(i + LQ < NI)
                    def _():
                        hi(hi_next, r, hi_slot).start(priority=0)

                if comp:
                    hi(old, r, old_slot).wait()
                    for m in range(NP):
                        v = _tree([
                            buf[old[0], stripe[m] + d * NP, old[1], pl.ds(r * KR, KR)]
                            .astype(F32).reshape(KR // 8, 8, 128)
                            for d in range(T // NP)])
                        for t in range(KR // 8):
                            ct = (8 * m + (KR // 8) * r + t) // WT
                            acc[ct] = acc[ct] + v[t]
            return tuple(acc)

        def steps(lo_i, hi_i, acc, **mode):
            return jax.lax.fori_loop(lo_i, hi_i, lambda i, a: step(i, a, **mode), acc)

        steps(0, CL, (), dma=True, drain=False, comp=False)
        acc = tuple(jnp.zeros((8, 128), F32) for _ in range(CT))
        acc = steps(CL, TABQ, acc, dma=True, drain=False, comp=True)

        cwd.wait()
        cwu.wait()
        wdt = wd_v[...].astype(F32)
        wd2_v[...] = wdt[:, T1 * 8:T2 * 8].astype(BF16)
        for c in range((CT - T2) * 8):
            wdc_v[c] = jnp.broadcast_to(wdt[:, T2 * 8 + c:T2 * 8 + c + 1], (R, 128))
        wut = wu_v[...].astype(F32).T
        for j in range(R):
            wub_v[j] = jnp.broadcast_to(wut[:, j:j + 1], (C, 128))

        acc = steps(TABQ, NI - DQ, acc, dma=True, drain=False, comp=True)
        acc = steps(NI - DQ, NI, acc, dma=True, drain=True, comp=True)
        acc = steps(NI, NI + CL, acc, dma=False, drain=False, comp=True)
        acc = list(acc)

        def add_fin(p, *copies):
            for c in copies:
                fin(*c).wait()
            v = _tree([buf[gi, st, MQ].astype(F32).reshape(8, 8, 128)
                       for st, g0, g1, _ in copies for gi in range(g0, g1)])
            for ct in sorted({(8 * p + i) // WT for i in range(8)}):
                acc[ct] = _tree([acc[ct]] + [v[i] for i in range(8)
                                             if (8 * p + i) // WT == ct])

        def means(t0, t1):
            a = jnp.stack(acc[t0:t1]).reshape((t1 - t0) * 8, 128)
            tot = jnp.sum(a, axis=1, keepdims=True)
            return jnp.broadcast_to(tot * inv_n, a.shape)

        for p in range(NP - 1):
            add_fin(p, (p, 0, G, p), (p + NP, 0, G, p + NP))
            if p == ST1:
                hp_v[...] = jnp.dot(wd_v[:, pl.ds(0, T1 * 8)], means(0, T1).astype(BF16),
                                    preferred_element_type=F32)
        m2_v[...] = means(T1, T2).astype(BF16)
        add_fin(NP - 1, (NP - 1, 0, G, NP - 1), (T - 1, 0, G - 1, T - 1))
        add_fin(NP - 1, (T - 1, G - 1, G, T))

        hp = hp_v[...] + jnp.dot(wd2_v[...], m2_v[...], preferred_element_type=F32)
        m3 = _rnd(means(T2, CT))
        h = _rnd(_tree([wdc_v[c] * m3[c:c + 1, :] for c in range((CT - T2) * 8)]) + hp)
        g = _rnd(h * _sigmoid(h))
        gb = [jnp.broadcast_to(g[j:j + 1, :], (8, 128)) for j in range(R)]

        scale = {}

        def scale_tile(ct):
            if ct not in scale:
                z = _tree([wub_v[j, pl.ds(ct * 8, 8), :] * gb[j] for j in range(R)])
                scale[ct] = _sigmoid(_rnd(z))
            return scale[ct]

        for p in range(NP):
            sc = jnp.stack([scale_tile((8 * p + i) // WT) for i in range(8)])
            for st in (p, p + NP):
                for gi in range(G):
                    v = buf[gi, st, 0].astype(F32).reshape(8, 8, 128)
                    buf[gi, st, 0] = (v * sc).reshape(RUN, 128).astype(BF16)
                pltpu.make_async_copy(buf.at[:, st, 0], o_hbm.at[:, st, 0], osem.at[p]).start()
            tab_v[p] = sc

        def wr(gi, st0, q, slot):
            s = (gi, pl.ds(st0, NA), q)
            return pltpu.make_async_copy(buf.at[s], o_hbm.at[s], osem.at[slot])

        def out_stripes(n, carry):
            gi = jax.lax.div(n, T // NA)
            st0 = jax.lax.rem(n, T // NA) * NA

            def out_run(q, carry):
                for a in range(NA):
                    v = buf[gi, st0 + a, q].astype(F32).reshape(8, 8, 128)
                    sc = tab_v[jax.lax.rem(st0 + a + q, NP)]
                    buf[gi, st0 + a, q] = (v * sc).reshape(RUN, 128).astype(BF16)
                slot = jax.lax.rem(q - 1, NP)
                wr(gi, st0, q, slot).wait()
                wr(gi, st0, q, slot).start()
                return carry

            return jax.lax.fori_loop(1, NQ, out_run, carry)

        jax.lax.fori_loop(0, NST // NA, out_stripes, 0)
        for p in range(NP):
            wr(G - 1, T - NA, NQ - NP + p, p).wait()

    xv = x.reshape(H, WT, 128, CT, 8).transpose(0, 3, 1, 4, 2).reshape(G, T, NQ, RUN, 128)
    out = pl.pallas_call(
        kernel,
        out_shape=jax.ShapeDtypeStruct(xv.shape, xv.dtype),
        in_specs=[pl.BlockSpec(memory_space=pl.ANY)] * 3,
        out_specs=pl.BlockSpec(memory_space=pl.ANY),
        scratch_shapes=[
            pltpu.VMEM(xv.shape, BF16),
            pltpu.VMEM((R, C), BF16),
            pltpu.VMEM((R, C), BF16),
            pltpu.VMEM((R, (T2 - T1) * 8), BF16),
            pltpu.VMEM(((CT - T2) * 8, R, 128), F32),
            pltpu.VMEM((R, C, 128), F32),
            pltpu.VMEM((R, 128), F32),
            pltpu.VMEM(((T2 - T1) * 8, 128), BF16),
            pltpu.VMEM((NP, 8, 8, 128), F32),
            pltpu.SemaphoreType.DMA((DQ * PPQ,)),
            pltpu.SemaphoreType.DMA((FQ * PPQ,)),
            pltpu.SemaphoreType.DMA((T + 1,)),
            pltpu.SemaphoreType.DMA((2,)),
            pltpu.SemaphoreType.DMA((NP,)),
        ],
        compiler_params=pltpu.CompilerParams(
            vmem_limit_bytes=64 * 1024 * 1024,
            disable_bounds_checks=True,
            disable_semaphore_checks=True,
        ),
    )(xv, w_down.T, w_up)
    return out.reshape(H, CT, WT, 8, 128).transpose(0, 2, 4, 1, 3).reshape(B, H, W, C)
```

```python
import jax
import jax.numpy as jnp
import jax.experimental.pallas as pl
import jax.experimental.pallas.tpu as pltpu

F32, BF16 = jnp.float32, jnp.bfloat16
_NEG_LOG2E = -1.4426950408889634


def _rnd(v):
    return v.astype(BF16).astype(F32)


def _sigmoid(v):
    d = _rnd(1.0 + _rnd(jnp.exp2(v * _NEG_LOG2E)))
    return _rnd(pl.reciprocal(d, approx=True))


def _tree(terms):
    terms = list(terms)
    while len(terms) > 1:
        nxt = [terms[i] + terms[i + 1] for i in range(0, len(terms) - 1, 2)]
        if len(terms) % 2:
            nxt.append(terms[-1])
        terms = nxt
    return terms[0]


@jax.jit
def pallas_standalone__se_block__vision_kernel(
    x: jax.Array,
    w_down: jax.Array,
    w_up: jax.Array,
):
    B, H, W, C = x.shape
    R = w_down.shape[1]
    CT, WT = C // 8, W // 128
    inv_n = 1.0 / (H * W)

    RUN = 64
    NQ = 64
    NP = CT * WT // 8
    NST = H * NP // NQ
    assert B == 1 and C % 8 == 0 and W % 128 == 0
    assert NP * 8 == CT * WT and NST * NQ == H * NP and NQ % NP == 1

    T, F = 2 * NP, 2
    G = NST // T
    PPQ = 4
    KR = RUN // PPQ
    MQ = NQ - 1
    NI = G * MQ
    DQ, LQ, CL = 6, 1, 2
    FQ = LQ + CL + 1
    TABQ = 40
    ST1 = 4
    T1 = 8 * (ST1 + 1) // WT
    T2 = 8 * (NP - 1) // WT
    NA = 2 * G
    assert G * T == NST and T % NA == 0
    assert LQ == 1 and DQ > PPQ and DQ * PPQ > NP

    def kernel(x_hbm, wd_hbm, wu_hbm, o_hbm,
               buf, wd_v, wu_v, wd2_v, wdc_v, wub_v, hp_v, m2_v, tab_v,
               bsem, fsem, lsem, wsem, osem):
        def split(i):
            return jax.lax.div(i, MQ), jax.lax.rem(i, MQ)

        def lo(gq, r, slot):
            s = (gq[0], pl.ds(0, T - F), gq[1], pl.ds(r * KR, KR))
            return pltpu.make_async_copy(x_hbm.at[s], buf.at[s], bsem.at[slot * PPQ + r])

        def hi(gq, r, slot):
            rows = slice(None) if r is None else pl.ds(r * KR, KR)
            s = (gq[0], pl.ds(T - F, F), gq[1], rows)
            return pltpu.make_async_copy(x_hbm.at[s], buf.at[s], fsem.at[slot])

        def fin(st, g0, g1, k):
            s = (pl.ds(g0, g1 - g0), st, MQ)
            return pltpu.make_async_copy(x_hbm.at[s], buf.at[s], lsem.at[k])

        for r in range(PPQ):
            lo((0, 0), r, 0).start(priority=1)

        def fill(j, carry):
            for r in range(PPQ):
                lo((0, j), r, j).start(priority=1)
            for r in range(PPQ):
                @pl.when(j == r + 1)
                def _():
                    hi((0, 0), r, 0).start(priority=0)
            return carry

        jax.lax.fori_loop(1, DQ, fill, 0)
        cwd = pltpu.make_async_copy(wd_hbm, wd_v, wsem.at[0])
        cwu = pltpu.make_async_copy(wu_hbm, wu_v, wsem.at[1])
        cwd.start()
        cwu.start()

        def add_runs(acc, p, runs):
            v = _tree([run.astype(F32).reshape(8, 8, 128) for run in runs])
            for ct in sorted({(8 * p + i) // WT for i in range(8)}):
                acc[ct] = _tree([acc[ct]] + [v[i] for i in range(8)
                                             if (8 * p + i) // WT == ct])

        def step(i, acc, *, dma, drain, comp):
            acc = list(acc)
            if dma:
                cur, lo_next, hi_next = split(i), split(i + DQ), split(i + LQ)
                lo_slot = jax.lax.rem(i, DQ)
                hi_slot = jax.lax.rem(i + LQ, FQ)
            if comp:
                old = split(i - CL)
                old_slot = jax.lax.rem(i - CL, FQ)
                q9 = jax.lax.rem(old[1], NP)
                stripe = [jnp.where(m < q9, m + NP - q9, m - q9) for m in range(NP)]
                hi(old, None, old_slot).wait()
            for r in range(PPQ):
                if dma:
                    lo(cur, r, lo_slot).wait()
                if dma and not drain:
                    lo(lo_next, r, lo_slot).start(priority=1)
                    hi(hi_next, r, hi_slot).start(priority=0)
                if dma and drain:
                    k = (i + DQ - NI) * PPQ + r

                    @pl.when(k < NP - 1)
                    def _():
                        fin(k, 0, G, k).start(priority=1)
                        fin(k + NP, 0, G, k + NP).start(priority=1)

                    if r == (NP - 1) % PPQ:
                        @pl.when(k == NP - 1)
                        def _():
                            fin(NP - 1, 0, G, NP - 1).start(priority=1)
                            fin(T - 1, 0, G - 1, T - 1).start(priority=1)

                    if r == NP % PPQ:
                        @pl.when(k == NP)
                        def _():
                            fin(T - 1, G - 1, G, T).start(priority=1)

                    @pl.when(i + LQ < NI)
                    def _():
                        hi(hi_next, r, hi_slot).start(priority=0)

                if comp:
                    for m in range(r * NP // PPQ, (r + 1) * NP // PPQ):
                        add_runs(acc, m, [buf[old[0], stripe[m] + d * NP, old[1]]
                                          for d in range(T // NP)])
            return tuple(acc)

        def steps(lo_i, hi_i, acc, **mode):
            return jax.lax.fori_loop(lo_i, hi_i, lambda i, a: step(i, a, **mode), acc)

        steps(0, CL, (), dma=True, drain=False, comp=False)
        acc = tuple(jnp.zeros((8, 128), F32) for _ in range(CT))
        acc = steps(CL, TABQ, acc, dma=True, drain=False, comp=True)

        cwd.wait()
        cwu.wait()
        wdt = wd_v[...].astype(F32)
        wd2_v[...] = wdt[:, T1 * 8:T2 * 8].astype(BF16)
        for c in range((CT - T2) * 8):
            wdc_v[c] = jnp.broadcast_to(wdt[:, T2 * 8 + c:T2 * 8 + c + 1], (R, 128))
        wut = wu_v[...].astype(F32).T
        for j in range(R):
            wub_v[j] = jnp.broadcast_to(wut[:, j:j + 1], (C, 128))

        acc = steps(TABQ, NI - DQ, acc, dma=True, drain=False, comp=True)
        acc = steps(NI - DQ, NI, acc, dma=True, drain=True, comp=True)
        acc = steps(NI, NI + CL, acc, dma=False, drain=False, comp=True)
        acc = list(acc)

        def add_fin(p, *copies):
            for c in copies:
                fin(*c).wait()
            add_runs(acc, p, [buf[gi, st, MQ] for st, g0, g1, _ in copies
                              for gi in range(g0, g1)])

        def means(t0, t1):
            a = jnp.stack(acc[t0:t1]).reshape((t1 - t0) * 8, 128)
            tot = jnp.sum(a, axis=1, keepdims=True)
            return jnp.broadcast_to(tot * inv_n, a.shape)

        for p in range(NP - 1):
            add_fin(p, (p, 0, G, p), (p + NP, 0, G, p + NP))
            if p == ST1:
                hp_v[...] = jnp.dot(wd_v[:, pl.ds(0, T1 * 8)], means(0, T1).astype(BF16),
                                    preferred_element_type=F32)
        m2_v[...] = means(T1, T2).astype(BF16)
        add_fin(NP - 1, (NP - 1, 0, G, NP - 1), (T - 1, 0, G - 1, T - 1))
        add_fin(NP - 1, (T - 1, G - 1, G, T))

        hp = hp_v[...] + jnp.dot(wd2_v[...], m2_v[...], preferred_element_type=F32)
        m3 = _rnd(means(T2, CT))
        h = _rnd(_tree([wdc_v[c] * m3[c:c + 1, :] for c in range((CT - T2) * 8)]) + hp)
        g = _rnd(h * _sigmoid(h))
        gb = [jnp.broadcast_to(g[j:j + 1, :], (8, 128)) for j in range(R)]

        scale = {}

        def scale_tile(ct):
            if ct not in scale:
                z = _tree([wub_v[j, pl.ds(ct * 8, 8), :] * gb[j] for j in range(R)])
                scale[ct] = _sigmoid(_rnd(z))
            return scale[ct]

        for p in range(NP):
            sc = jnp.stack([scale_tile((8 * p + i) // WT) for i in range(8)])
            for st in (p, p + NP):
                for gi in range(G):
                    v = buf[gi, st, 0].astype(F32).reshape(8, 8, 128)
                    buf[gi, st, 0] = (v * sc).reshape(RUN, 128).astype(BF16)
                pltpu.make_async_copy(buf.at[:, st, 0], o_hbm.at[:, st, 0], osem.at[p]).start()
            tab_v[p] = sc
            if p < NA - 1:
                tab_v[p + NP] = sc

        def wr(gi, st0, q, slot):
            s = (gi, pl.ds(st0, NA), q)
            return pltpu.make_async_copy(buf.at[s], o_hbm.at[s], osem.at[slot])

        def out_stripes(n, carry):
            gi = jax.lax.div(n, T // NA)
            st0 = jax.lax.rem(n, T // NA) * NA

            def out_run(q, carry):
                s = (gi, pl.ds(st0, NA), q)
                sc = tab_v[pl.ds(jax.lax.rem(st0 + q, NP), NA)]
                v = buf[s].astype(F32).reshape(NA, 8, 8, 128)
                buf[s] = (v * sc).reshape(NA, RUN, 128).astype(BF16)
                slot = jax.lax.rem(q - 1, NP)
                wr(gi, st0, q, slot).wait()
                wr(gi, st0, q, slot).start()
                return carry

            return jax.lax.fori_loop(1, NQ, out_run, carry)

        jax.lax.fori_loop(0, NST // NA, out_stripes, 0)
        for p in range(NP):
            wr(G - 1, T - NA, NQ - NP + p, p).wait()

    xv = x.reshape(H, WT, 128, CT, 8).transpose(0, 3, 1, 4, 2).reshape(G, T, NQ, RUN, 128)
    out = pl.pallas_call(
        kernel,
        out_shape=jax.ShapeDtypeStruct(xv.shape, xv.dtype),
        in_specs=[pl.BlockSpec(memory_space=pl.ANY)] * 3,
        out_specs=pl.BlockSpec(memory_space=pl.ANY),
        scratch_shapes=[
            pltpu.VMEM(xv.shape, BF16),
            pltpu.VMEM((R, C), BF16),
            pltpu.VMEM((R, C), BF16),
            pltpu.VMEM((R, (T2 - T1) * 8), BF16),
            pltpu.VMEM(((CT - T2) * 8, R, 128), F32),
            pltpu.VMEM((R, C, 128), F32),
            pltpu.VMEM((R, 128), F32),
            pltpu.VMEM(((T2 - T1) * 8, 128), BF16),
            pltpu.VMEM((NP + NA - 1, 8, 8, 128), F32),
            pltpu.SemaphoreType.DMA((DQ * PPQ,)),
            pltpu.SemaphoreType.DMA((FQ,)),
            pltpu.SemaphoreType.DMA((T + 1,)),
            pltpu.SemaphoreType.DMA((2,)),
            pltpu.SemaphoreType.DMA((NP,)),
        ],
        compiler_params=pltpu.CompilerParams(
            vmem_limit_bytes=64 * 1024 * 1024,
            disable_bounds_checks=True,
            disable_semaphore_checks=True,
        ),
    )(xv, w_down.T, w_up)
    return out.reshape(H, CT, WT, 8, 128).transpose(0, 2, 4, 1, 3).reshape(B, H, W, C)
```
